```python
import os as _os
_os.environ.setdefault("JAX_PLATFORMS", "cpu")
import jax
import jax.numpy as jnp

def _softmax(x, axis=-1):
    return jax.nn.softmax(x, axis=axis)
def _gelu(x):
    return jax.nn.gelu(x, approximate=True)
def _silu(x):
    return jax.nn.silu(x)
def _sigmoid(x):
    return jax.nn.sigmoid(x)
def _layernorm(x, axis=-1, eps=1e-5):
    m = jnp.mean(x, axis=axis, keepdims=True)
    v = jnp.var(x, axis=axis, keepdims=True)
    return (x - m) / jnp.sqrt(v + eps)
def _scatter_add(tgt, idx, src, axis=0):
    return tgt.at[idx].add(src)
def _segment_sum(src, seg, n):
    return jax.ops.segment_sum(src, seg, n)
class _Rng:
    def __init__(self, key):
        self._k = key
    def _next(self):
        self._k, sub = jax.random.split(self._k)
        return sub
    def normal(self, shape):
        return jax.random.normal(self._next(), shape, dtype=jnp.bfloat16)
    def randint(self, lo, hi, shape):
        return jax.random.randint(self._next(), shape, lo, hi, dtype=jnp.int32)
    def uniform(self, shape, lo=0.0, hi=1.0):
        return jax.random.uniform(self._next(), shape, jnp.bfloat16, lo, hi)
    def permutation(self, n):
        return jax.random.permutation(self._next(), n)


kernel_name = 'interleave_layers__gqa_block_cached__dense_activation_mish__decode'

def setup_inputs():
    _rng = _Rng(jax.random.key(int.from_bytes(__import__("os").urandom(4), "little")))
    _w = (lambda a: (lambda t: t.astype(jnp.bfloat16) if jnp.issubdtype(t.dtype, jnp.floating) else t)(jnp.asarray(a)))
    def _A_setup():
        B, Sq, D = 1, 1, 512
        Hq, Hkv, Sk, Dh = 32, 8, 65536, 128
        assert Hq % Hkv == 0, (Hq, Hkv)
        return {
            "x": _w((lambda *s: _rng.normal(s) * 0.05)(B, Sq, D)),
            "k_cache": _w((lambda *s: _rng.normal(s) * 1.6)(B, Hkv, Sk, Dh)),
            "v_cache": _w((lambda *s: _rng.normal(s) * 1.6)(B, Hkv, Sk, Dh)),
            "wq": _w((lambda *s: _rng.normal(s) * 1.6)(D, Hq * Dh) * (D ** -0.5)),
            "wo": _w((lambda *s: _rng.normal(s) * 1.6)(Hq * Dh, D) * ((Hq * Dh) ** -0.5)),
        }
    _A_in = _A_setup()

    def _B_setup():
        B, S, D, F = 1, 1, 512, 1792
        return {
            "x": _w((lambda *s: _rng.normal(s) * 0.05)(B, S, D)),
            "w1": _w((lambda *s: _rng.normal(s) * 0.8)(D, F) * (D ** -0.5)),
            "b1": _w((lambda *s: _rng.normal(s) * 0.8)(F)),
            "w2": _w((lambda *s: _rng.normal(s) * 0.8)(F, D) * (F ** -0.5)),
        }
    _B_in = _B_setup()

    return {
        "A_x": _A_in["x"],
        "A_k_cache": _A_in["k_cache"],
        "A_v_cache": _A_in["v_cache"],
        "A_wq": _A_in["wq"],
        "A_wo": _A_in["wo"],
        "B_x": _B_in["x"],
        "B_w1": _B_in["w1"],
        "B_b1": _B_in["b1"],
        "B_w2": _B_in["w2"],
    }

def reference(A_x, A_k_cache, A_v_cache, A_wq, A_wo, B_x, B_w1, B_b1, B_w2):
    def _A_ref(x, k_cache, v_cache, wq, wo):
        B, Sq, D = x.shape
        Hq, Dh = 32, 128
        Hkv = k_cache.shape[1]
        rep = Hq // Hkv
        q = (lambda x, *d: x.transpose(*d))((x @ wq).reshape(B, Sq, Hq, Dh), 0, 2, 1, 3)
        k = jnp.repeat(k_cache, rep, axis=1)
        v = jnp.repeat(v_cache, rep, axis=1)
        scores = jnp.einsum("bhqd,bhkd->bhqk", q, k) * (Dh ** -0.5)
        p = _softmax(scores, axis=-1)
        o = jnp.einsum("bhqk,bhkd->bhqd", p, v)
        return (lambda x, *d: x.transpose(*d))(o, 0, 2, 1, 3).reshape(B, Sq, Hq * Dh) @ wo

    def _B_ref(x, w1, b1, w2):
        h = jnp.einsum("bsd,df->bsf", x, w1) + b1
        sp = jnp.log1p(jnp.exp(-jnp.abs(h))) + jnp.where(h > 0, h, jnp.zeros_like(h))
        act = h * jnp.tanh(sp)
        return jnp.einsum("bsf,fd->bsd", act, w2)

    x = A_x
    x = x + _A_ref(_layernorm(x, axis=-1), A_k_cache, A_v_cache, A_wq, A_wo)
    x = x + _B_ref(_layernorm(x, axis=-1), B_w1, B_b1, B_w2)
    x = x + _A_ref(_layernorm(x, axis=-1), A_k_cache, A_v_cache, A_wq, A_wo)
    x = x + _B_ref(_layernorm(x, axis=-1), B_w1, B_b1, B_w2)
    return x
```

```python
import functools

import jax
import jax.numpy as jnp
import jax.experimental.pallas as pl
import jax.experimental.pallas.tpu as pltpu

_NT = (((1,), (1,)), ((), ()))
_NN = (((1,), (0,)), ((), ()))

_HQ, _HKV, _SK, _DH = 32, 8, 65536, 128
_REP = _HQ // _HKV
_D, _F = 512, 1792
_BK = 4096
_BPH = _SK // _BK
_T = _HKV * _BPH
_NRING = 4
_NRES = 53
_NSTR = _T - _NRES
_RPS = -(-_NRES // _NSTR)


def _layernorm(x):
    m = jnp.mean(x, axis=-1, keepdims=True)
    xc = x - m
    v = jnp.mean(xc * xc, axis=-1, keepdims=True)
    return xc / jnp.sqrt(v + 1e-5)


def _kernel(x_ref, b1_ref, k_hbm, v_hbm, wq_hbm, wo_hbm, w1_hbm, w2_hbm, o_ref,
            kpool, vpool, wq_v, wo_v, w1_v, w2_v,
            q_s, m_s, l_s, acc_s, row_s, kv_sems, w_sems):
    scale = _DH ** -0.5

    def w_copy(i):
        src, dst = ((wq_hbm, wq_v), (wo_hbm, wo_v), (w1_hbm, w1_v), (w2_hbm, w2_v))[i]
        return pltpu.make_async_copy(src, dst, w_sems.at[i])

    def kv_copies(blk, slot, sem):
        row0 = pl.multiple_of(blk * _BK, _BK)
        return (
            pltpu.make_async_copy(k_hbm.at[pl.ds(row0, _BK)], kpool.at[slot], kv_sems.at[0, sem]),
            pltpu.make_async_copy(v_hbm.at[pl.ds(row0, _BK)], vpool.at[slot], kv_sems.at[1, sem]),
        )

    def load_desc(j):
        blk = jnp.where(j >= _T, j - _T, j)
        slot = jnp.where(
            j >= _T, (j - _T) % _NRING,
            jnp.where(j < _NSTR, j % _NRING, _NRING + (j - _NSTR)))
        return blk, slot

    def start_load(j):
        blk, slot = load_desc(j)
        for c in kv_copies(blk, slot, j % _NRING):
            c.start()

    def wait_load(j):
        blk, slot = load_desc(j)
        for c in kv_copies(blk, slot, j % _NRING):
            c.wait()

    def attend(blk, slot):
        h = blk // _BPH
        k = kpool[slot]
        v = vpool[slot]
        q = q_s[h]
        s = jax.lax.dot_general(q, k, _NT, preferred_element_type=jnp.float32) * scale
        m_old = m_s[h]
        m_new = jnp.maximum(m_old, jnp.max(s, axis=-1, keepdims=True))
        alpha = jnp.exp(m_old - m_new)
        p = jnp.exp(s - m_new)
        l_s[h] = l_s[h] * alpha + jnp.sum(p, axis=-1, keepdims=True)
        acc_s[h] = acc_s[h] * alpha + jax.lax.dot_general(
            p.astype(jnp.bfloat16), v, _NN, preferred_element_type=jnp.float32)
        m_s[h] = m_new

    def start_layer(x):
        xn = _layernorm(x).astype(jnp.bfloat16)
        q = jnp.dot(xn, wq_v[...], preferred_element_type=jnp.float32)
        q = q.astype(jnp.bfloat16)
        q_s[...] = jnp.zeros(q_s.shape, q_s.dtype)
        for h in range(_HKV):
            for r in range(_REP):
                j = h * _REP + r
                q_s[h, r:r + 1, :] = q[:, j * _DH:(j + 1) * _DH]
        m_s[...] = jnp.full(m_s.shape, -jnp.inf, jnp.float32)
        l_s[...] = jnp.zeros(l_s.shape, jnp.float32)
        acc_s[...] = jnp.zeros(acc_s.shape, jnp.float32)

    def finish_layer(x):
        for h in range(_HKV):
            o = acc_s[h] / l_s[h]
            for r in range(_REP):
                j = h * _REP + r
                row_s[:, j * _DH:(j + 1) * _DH] = o[r:r + 1, :]
        o = row_s[...].astype(jnp.bfloat16)
        x = x + jnp.dot(o, wo_v[...], preferred_element_type=jnp.float32)
        xn = _layernorm(x).astype(jnp.bfloat16)
        hh = jnp.dot(xn, w1_v[...], preferred_element_type=jnp.float32) + b1_ref[...].astype(jnp.float32)
        sp = jnp.log1p(jnp.exp(-jnp.abs(hh))) + jnp.maximum(hh, 0.0)
        act = (hh * jnp.tanh(sp)).astype(jnp.bfloat16)
        return x + jnp.dot(act, w2_v[...], preferred_element_type=jnp.float32)

    w_copy(0).start()
    for j in range(_NRING):
        start_load(j)
    for i in range(1, 4):
        w_copy(i).start()

    x0 = x_ref[...].astype(jnp.float32)
    w_copy(0).wait()
    start_layer(x0)

    def pass1(t, c):
        wait_load(t)
        blk, slot = load_desc(t)
        attend(blk, slot)
        start_load(t + _NRING)
        return c

    jax.lax.fori_loop(0, _T, pass1, 0)

    for i in range(1, 4):
        w_copy(i).wait()
    x1 = finish_layer(x0)
    start_layer(x1)

    def pass2(k, c):
        j = _T + k
        wait_load(j)
        attend(k, k % _NRING)

        @pl.when(k + _NRING < _NSTR)
        def _():
            start_load(j + _NRING)

        for i in range(_RPS):
            r = k * _RPS + i

            @pl.when(r < _NRES)
            def _():
                attend(_NSTR + r, _NRING + r)
        return c

    jax.lax.fori_loop(0, _NSTR, pass2, 0)

    x2 = finish_layer(x1)
    o_ref[...] = x2.astype(o_ref.dtype)


@jax.jit
def pallas_interleave_layers__gqa_block_cached__dense_activation_mish__decode_kernel(
    A_x: jax.Array,
    A_k_cache: jax.Array,
    A_v_cache: jax.Array,
    A_wq: jax.Array,
    A_wo: jax.Array,
    B_x: jax.Array,
    B_w1: jax.Array,
    B_b1: jax.Array,
    B_w2: jax.Array,
):
    del B_x
    x = A_x.reshape(1, _D)
    k = A_k_cache.reshape(_HKV * _SK, _DH)
    v = A_v_cache.reshape(_HKV * _SK, _DH)
    b1 = B_b1.reshape(1, _F)
    nslot = _NRING + _NRES
    hbm = pl.BlockSpec(memory_space=pl.ANY)
    vmem = pl.BlockSpec(memory_space=pltpu.VMEM)
    out = pl.pallas_call(
        _kernel,
        out_shape=jax.ShapeDtypeStruct((1, _D), A_x.dtype),
        in_specs=[vmem, vmem, hbm, hbm, hbm, hbm, hbm, hbm],
        out_specs=vmem,
        scratch_shapes=[
            pltpu.VMEM((nslot, _BK, _DH), jnp.bfloat16),
            pltpu.VMEM((nslot, _BK, _DH), jnp.bfloat16),
            pltpu.VMEM((_D, _HQ * _DH), jnp.bfloat16),
            pltpu.VMEM((_HQ * _DH, _D), jnp.bfloat16),
            pltpu.VMEM((_D, _F), jnp.bfloat16),
            pltpu.VMEM((_F, _D), jnp.bfloat16),
            pltpu.VMEM((_HKV, 8, _DH), jnp.bfloat16),
            pltpu.VMEM((_HKV, 8, 1), jnp.float32),
            pltpu.VMEM((_HKV, 8, 1), jnp.float32),
            pltpu.VMEM((_HKV, 8, _DH), jnp.float32),
            pltpu.VMEM((1, _HQ * _DH), jnp.float32),
            pltpu.SemaphoreType.DMA((2, _NRING)),
            pltpu.SemaphoreType.DMA((4,)),
        ],
        compiler_params=pltpu.CompilerParams(vmem_limit_bytes=128 * 1024 * 1024),
    )(x, b1, k, v, A_wq, A_wo, B_w1, B_w2)
    return out.reshape(A_x.shape)
```

```python
import jax
import jax.numpy as jnp
import jax.experimental.pallas as pl
import jax.experimental.pallas.tpu as pltpu

_NT = (((1,), (1,)), ((), ()))
_NN = (((1,), (0,)), ((), ()))

_HQ, _HKV, _SK, _DH = 32, 8, 65536, 128
_REP = _HQ // _HKV
_D, _F = 512, 1792
_BK = 2048
_BPH = _SK // _BK
_T = _HKV * _BPH
_NRING = 2
_NRES = 114
_NSTR = _T - _NRES
_RPS = -(-_NRES // _NSTR)


def _layernorm(x):
    m = jnp.mean(x, axis=-1, keepdims=True)
    xc = x - m
    v = jnp.mean(xc * xc, axis=-1, keepdims=True)
    return xc / jnp.sqrt(v + 1e-5)


def _kernel(x_hbm, b1_hbm, k_hbm, v_hbm, wq_hbm, wo_hbm, w1_hbm, w2_hbm, o_ref,
            kpool, vpool, wq_v, wo_v, w1_v, w2_v, x_v, b1_v,
            q_s, m_s, l_s, acc_s, row_s, proj_s, cnt_s, kv_sems, w_sems):
    scale = _DH ** -0.5
    i_wq, i_wo, i_w1, i_w2, i_x, i_b1 = range(6)

    def w_copy(i):
        src, dst = ((wq_hbm, wq_v), (wo_hbm, wo_v), (w1_hbm, w1_v),
                    (w2_hbm, w2_v), (x_hbm, x_v), (b1_hbm, b1_v))[i]
        return pltpu.make_async_copy(src, dst, w_sems.at[i])

    def load_desc(j):
        blk = jnp.where(j >= _T, j - _T, j)
        slot = jnp.where(
            j >= _T, (j - _T) % _NRING,
            jnp.where(j < _NSTR, j % _NRING, _NRING + (j - _NSTR)))
        return blk, slot

    def kv_copies(j):
        blk, slot = load_desc(j)
        sem = j % _NRING
        row0 = pl.multiple_of(blk * _BK, _BK)
        return (
            pltpu.make_async_copy(k_hbm.at[pl.ds(row0, _BK)], kpool.at[slot], kv_sems.at[0, sem]),
            pltpu.make_async_copy(v_hbm.at[pl.ds(row0, _BK)], vpool.at[slot], kv_sems.at[1, sem]),
        )

    def start_load(j):
        for c in kv_copies(j):
            c.start()

    def wait_load(j):
        for c in kv_copies(j):
            c.wait()

    def project(h):
        o = acc_s[h] / l_s[h]
        for r in range(_REP):
            row_s[:, r * _DH:(r + 1) * _DH] = o[r:r + 1, :]
        o = row_s[...].astype(jnp.bfloat16)
        r0 = pl.multiple_of(h * (_REP * _DH), _REP * _DH)
        proj_s[...] += jnp.dot(o, wo_v[pl.ds(r0, _REP * _DH), :],
                               preferred_element_type=jnp.float32)

    def attend(blk, slot):
        h = blk // _BPH
        k = kpool[slot]
        v = vpool[slot]
        q = q_s[h]
        s = jax.lax.dot_general(q, k, _NT, preferred_element_type=jnp.float32) * scale
        m_old = m_s[h]
        m_new = jnp.maximum(m_old, jnp.max(s, axis=-1, keepdims=True))
        alpha = jnp.exp(m_old - m_new)
        p = jnp.exp(s - m_new)
        l_s[h] = l_s[h] * alpha + jnp.sum(p, axis=-1, keepdims=True)
        acc_s[h] = acc_s[h] * alpha + jax.lax.dot_general(
            p.astype(jnp.bfloat16), v, _NN, preferred_element_type=jnp.float32)
        m_s[h] = m_new
        c = cnt_s[h] + 1
        cnt_s[h] = c

        @pl.when(c == _BPH)
        def _():
            project(h)

    def start_layer(x):
        xn = _layernorm(x).astype(jnp.bfloat16)
        q = jnp.dot(xn, wq_v[...], preferred_element_type=jnp.float32)
        q = q.astype(jnp.bfloat16)
        q_s[...] = jnp.zeros(q_s.shape, q_s.dtype)
        for h in range(_HKV):
            for r in range(_REP):
                j = h * _REP + r
                q_s[h, r:r + 1, :] = q[:, j * _DH:(j + 1) * _DH]
        m_s[...] = jnp.full(m_s.shape, -jnp.inf, jnp.float32)
        l_s[...] = jnp.zeros(l_s.shape, jnp.float32)
        acc_s[...] = jnp.zeros(acc_s.shape, jnp.float32)
        proj_s[...] = jnp.zeros(proj_s.shape, jnp.float32)
        for h in range(_HKV):
            cnt_s[h] = 0

    def finish_layer(x, first):
        x = x + proj_s[...]
        xn = _layernorm(x).astype(jnp.bfloat16)
        if first:
            w_copy(i_w1).wait()
            start_load(_T + _NRING - 2)
        b1 = b1_v[...].astype(jnp.float32).reshape(1, _F)
        hh = jnp.dot(xn, w1_v[...], preferred_element_type=jnp.float32) + b1
        sp = jnp.log1p(jnp.exp(-jnp.abs(hh))) + jnp.maximum(hh, 0.0)
        act = (hh * jnp.tanh(sp)).astype(jnp.bfloat16)
        if first:
            w_copy(i_w2).wait()
            start_load(_T + _NRING - 1)
        return x + jnp.dot(act, w2_v[...], preferred_element_type=jnp.float32)

    w_copy(i_x).start()
    w_copy(i_wq).start()
    for j in range(_NRING):
        start_load(j)
    w_copy(i_wo).start()
    w_copy(i_b1).start()

    w_copy(i_x).wait()
    x0 = x_v[...].astype(jnp.float32)
    w_copy(i_wq).wait()
    start_layer(x0)

    def pass1(t, c):
        @pl.when(t == _BPH - 1)
        def _():
            w_copy(i_wo).wait()
            w_copy(i_b1).wait()

        wait_load(t)
        blk, slot = load_desc(t)
        attend(blk, slot)
        jn = t + _NRING

        @pl.when(jn < _T)
        def _():
            start_load(jn)

        @pl.when(jn == _T)
        def _():
            w_copy(i_w1).start()

        @pl.when(jn == _T + 1)
        def _():
            w_copy(i_w2).start()

        if _NRING > 2:
            @pl.when(jn >= _T + 2)
            def _():
                start_load(jn - 2)
        return c

    jax.lax.fori_loop(0, _T, pass1, 0)

    x1 = finish_layer(x0, True)
    start_layer(x1)

    def pass2(k, c):
        j = _T + k
        wait_load(j)
        attend(k, k % _NRING)

        @pl.when(k + _NRING < _NSTR)
        def _():
            start_load(j + _NRING)

        for i in range(_RPS):
            r = k * _RPS + i

            @pl.when(r < _NRES)
            def _():
                attend(_NSTR + r, _NRING + r)
        return c

    jax.lax.fori_loop(0, _NSTR, pass2, 0)

    x2 = finish_layer(x1, False)
    o_ref[...] = x2.astype(o_ref.dtype)


@jax.jit
def pallas_interleave_layers__gqa_block_cached__dense_activation_mish__decode_kernel(
    A_x: jax.Array,
    A_k_cache: jax.Array,
    A_v_cache: jax.Array,
    A_wq: jax.Array,
    A_wo: jax.Array,
    B_x: jax.Array,
    B_w1: jax.Array,
    B_b1: jax.Array,
    B_w2: jax.Array,
):
    del B_x
    x = A_x.reshape(1, _D)
    k = A_k_cache.reshape(_HKV * _SK, _DH)
    v = A_v_cache.reshape(_HKV * _SK, _DH)
    nslot = _NRING + _NRES
    hbm = pl.BlockSpec(memory_space=pl.ANY)
    out = pl.pallas_call(
        _kernel,
        out_shape=jax.ShapeDtypeStruct((1, _D), A_x.dtype),
        in_specs=[hbm] * 8,
        out_specs=pl.BlockSpec(memory_space=pltpu.VMEM),
        scratch_shapes=[
            pltpu.VMEM((nslot, _BK, _DH), jnp.bfloat16),
            pltpu.VMEM((nslot, _BK, _DH), jnp.bfloat16),
            pltpu.VMEM((_D, _HQ * _DH), jnp.bfloat16),
            pltpu.VMEM((_HQ * _DH, _D), jnp.bfloat16),
            pltpu.VMEM((_D, _F), jnp.bfloat16),
            pltpu.VMEM((_F, _D), jnp.bfloat16),
            pltpu.VMEM((1, _D), jnp.bfloat16),
            pltpu.VMEM((_F,), jnp.bfloat16),
            pltpu.VMEM((_HKV, 8, _DH), jnp.bfloat16),
            pltpu.VMEM((_HKV, 8, 1), jnp.float32),
            pltpu.VMEM((_HKV, 8, 1), jnp.float32),
            pltpu.VMEM((_HKV, 8, _DH), jnp.float32),
            pltpu.VMEM((1, _REP * _DH), jnp.float32),
            pltpu.VMEM((1, _D), jnp.float32),
            pltpu.SMEM((_HKV,), jnp.int32),
            pltpu.SemaphoreType.DMA((2, _NRING)),
            pltpu.SemaphoreType.DMA((6,)),
        ],
        compiler_params=pltpu.CompilerParams(vmem_limit_bytes=128 * 1024 * 1024),
    )(x, B_b1, k, v, A_wq, A_wo, B_w1, B_w2)
    return out.reshape(A_x.shape)
```

```python
import jax
import jax.numpy as jnp
import jax.experimental.pallas as pl
import jax.experimental.pallas.tpu as pltpu

_NT = (((1,), (1,)), ((), ()))
_NN = (((1,), (0,)), ((), ()))

_HQ, _HKV, _SK, _DH = 32, 8, 65536, 128
_REP = _HQ // _HKV
_D, _F = 512, 1792
_BK = 2048
_BPH = _SK // _BK
_T = _HKV * _BPH
_NRING = 2
_NRES = 114
_NSTR = _T - _NRES
_RPS = -(-_NRES // _NSTR)


def _layernorm(x):
    m = jnp.mean(x, axis=-1, keepdims=True)
    xc = x - m
    v = jnp.mean(xc * xc, axis=-1, keepdims=True)
    return xc / jnp.sqrt(v + 1e-5)


def _kernel(x_hbm, b1_hbm, k_hbm, v_hbm, wq_hbm, wo_hbm, w1_hbm, w2_hbm, o_ref,
            kpool, vpool, wq_v, wo_v, w1_v, w2_v, x_v, b1_v,
            q_s, m_s, l_s, acc_s, row_s, proj_s, cnt_s, kv_sems, w_sems):
    scale = _DH ** -0.5
    i_wq, i_wo, i_w1, i_w2, i_x, i_b1 = range(6)

    def w_copy(i):
        src, dst = ((wq_hbm, wq_v), (wo_hbm, wo_v), (w1_hbm, w1_v),
                    (w2_hbm, w2_v), (x_hbm, x_v), (b1_hbm, b1_v))[i]
        return pltpu.make_async_copy(src, dst, w_sems.at[i])

    def load_desc(j):
        blk = jnp.where(j >= _T, j - _T, j)
        slot = jnp.where(
            j >= _T, (j - _T) % _NRING,
            jnp.where(j < _NSTR, j % _NRING, _NRING + (j - _NSTR)))
        return blk, slot

    def kv_copy(j, which):
        blk, slot = load_desc(j)
        src, dst = ((k_hbm, kpool), (v_hbm, vpool))[which]
        row0 = pl.multiple_of(blk * _BK, _BK)
        return pltpu.make_async_copy(
            src.at[pl.ds(row0, _BK)], dst.at[slot], kv_sems.at[which, j % _NRING])

    def start_load(j):
        kv_copy(j, 0).start()
        kv_copy(j, 1).start()

    def project(h):
        o = acc_s[h] / l_s[h]
        for r in range(_REP):
            row_s[:, r * _DH:(r + 1) * _DH] = o[r:r + 1, :]
        o = row_s[...].astype(jnp.bfloat16)
        r0 = pl.multiple_of(h * (_REP * _DH), _REP * _DH)
        proj_s[...] += jnp.dot(o, wo_v[pl.ds(r0, _REP * _DH), :],
                               preferred_element_type=jnp.float32)

    def attend(blk, slot, j=None):
        h = blk // _BPH
        if j is not None:
            kv_copy(j, 0).wait()
        k = kpool[slot]
        q = q_s[h]
        s = jax.lax.dot_general(q, k, _NT, preferred_element_type=jnp.float32) * scale
        m_old = m_s[h]
        m_new = jnp.maximum(m_old, jnp.max(s, axis=-1, keepdims=True))
        alpha = jnp.exp(m_old - m_new)
        p = jnp.exp(s - m_new)
        l_s[h] = l_s[h] * alpha + jnp.sum(p, axis=-1, keepdims=True)
        if j is not None:
            kv_copy(j, 1).wait()
        v = vpool[slot]
        acc_s[h] = acc_s[h] * alpha + jax.lax.dot_general(
            p.astype(jnp.bfloat16), v, _NN, preferred_element_type=jnp.float32)
        m_s[h] = m_new
        c = cnt_s[h] + 1
        cnt_s[h] = c

        @pl.when(c == _BPH)
        def _():
            project(h)

    def start_layer(x):
        xn = _layernorm(x).astype(jnp.bfloat16)
        q = jnp.dot(xn, wq_v[...], preferred_element_type=jnp.float32)
        q = q.astype(jnp.bfloat16)
        q_s[...] = jnp.zeros(q_s.shape, q_s.dtype)
        for h in range(_HKV):
            for r in range(_REP):
                j = h * _REP + r
                q_s[h, r:r + 1, :] = q[:, j * _DH:(j + 1) * _DH]
        m_s[...] = jnp.full(m_s.shape, -jnp.inf, jnp.float32)
        l_s[...] = jnp.zeros(l_s.shape, jnp.float32)
        acc_s[...] = jnp.zeros(acc_s.shape, jnp.float32)
        proj_s[...] = jnp.zeros(proj_s.shape, jnp.float32)
        for h in range(_HKV):
            cnt_s[h] = 0

    def finish_layer(x, first):
        x = x + proj_s[...]
        xn = _layernorm(x).astype(jnp.bfloat16)
        if first:
            w_copy(i_w1).wait()
            start_load(_T + _NRING - 2)
        b1 = b1_v[...].astype(jnp.float32).reshape(1, _F)
        hh = jnp.dot(xn, w1_v[...], preferred_element_type=jnp.float32) + b1
        sp = jnp.log1p(jnp.exp(-jnp.abs(hh))) + jnp.maximum(hh, 0.0)
        act = (hh * jnp.tanh(sp)).astype(jnp.bfloat16)
        if first:
            w_copy(i_w2).wait()
            start_load(_T + _NRING - 1)
        return x + jnp.dot(act, w2_v[...], preferred_element_type=jnp.float32)

    w_copy(i_x).start()
    w_copy(i_wq).start()
    for j in range(_NRING):
        start_load(j)
    w_copy(i_wo).start()
    w_copy(i_b1).start()

    w_copy(i_x).wait()
    x0 = x_v[...].astype(jnp.float32)
    w_copy(i_wq).wait()
    start_layer(x0)

    def pass1(t, c):
        @pl.when(t == _BPH - 1)
        def _():
            w_copy(i_wo).wait()
            w_copy(i_b1).wait()

        blk, slot = load_desc(t)
        attend(blk, slot, t)
        jn = t + _NRING

        @pl.when(jn < _T)
        def _():
            start_load(jn)

        @pl.when(jn == _T)
        def _():
            w_copy(i_w1).start()

        @pl.when(jn == _T + 1)
        def _():
            w_copy(i_w2).start()

        if _NRING > 2:
            @pl.when(jn >= _T + 2)
            def _():
                start_load(jn - 2)
        return c

    jax.lax.fori_loop(0, _T, pass1, 0)

    x1 = finish_layer(x0, True)
    start_layer(x1)

    def pass2(k, c):
        j = _T + k
        attend(k, k % _NRING, j)

        @pl.when(k + _NRING < _NSTR)
        def _():
            start_load(j + _NRING)

        for i in range(_RPS):
            r = k * _RPS + i

            @pl.when(r < _NRES)
            def _():
                attend(_NSTR + r, _NRING + r)
        return c

    jax.lax.fori_loop(0, _NSTR, pass2, 0)

    x2 = finish_layer(x1, False)
    o_ref[...] = x2.astype(o_ref.dtype)


@jax.jit
def pallas_interleave_layers__gqa_block_cached__dense_activation_mish__decode_kernel(
    A_x: jax.Array,
    A_k_cache: jax.Array,
    A_v_cache: jax.Array,
    A_wq: jax.Array,
    A_wo: jax.Array,
    B_x: jax.Array,
    B_w1: jax.Array,
    B_b1: jax.Array,
    B_w2: jax.Array,
):
    del B_x
    x = A_x.reshape(1, _D)
    k = A_k_cache.reshape(_HKV * _SK, _DH)
    v = A_v_cache.reshape(_HKV * _SK, _DH)
    nslot = _NRING + _NRES
    hbm = pl.BlockSpec(memory_space=pl.ANY)
    out = pl.pallas_call(
        _kernel,
        out_shape=jax.ShapeDtypeStruct((1, _D), A_x.dtype),
        in_specs=[hbm] * 8,
        out_specs=pl.BlockSpec(memory_space=pltpu.VMEM),
        scratch_shapes=[
            pltpu.VMEM((nslot, _BK, _DH), jnp.bfloat16),
            pltpu.VMEM((nslot, _BK, _DH), jnp.bfloat16),
            pltpu.VMEM((_D, _HQ * _DH), jnp.bfloat16),
            pltpu.VMEM((_HQ * _DH, _D), jnp.bfloat16),
            pltpu.VMEM((_D, _F), jnp.bfloat16),
            pltpu.VMEM((_F, _D), jnp.bfloat16),
            pltpu.VMEM((1, _D), jnp.bfloat16),
            pltpu.VMEM((_F,), jnp.bfloat16),
            pltpu.VMEM((_HKV, 8, _DH), jnp.bfloat16),
            pltpu.VMEM((_HKV, 8, 1), jnp.float32),
            pltpu.VMEM((_HKV, 8, 1), jnp.float32),
            pltpu.VMEM((_HKV, 8, _DH), jnp.float32),
            pltpu.VMEM((1, _REP * _DH), jnp.float32),
            pltpu.VMEM((1, _D), jnp.float32),
            pltpu.SMEM((_HKV,), jnp.int32),
            pltpu.SemaphoreType.DMA((2, _NRING)),
            pltpu.SemaphoreType.DMA((6,)),
        ],
        compiler_params=pltpu.CompilerParams(vmem_limit_bytes=128 * 1024 * 1024),
    )(x, B_b1, k, v, A_wq, A_wo, B_w1, B_w2)
    return out.reshape(A_x.shape)
```

```python
import jax
import jax.numpy as jnp
import jax.experimental.pallas as pl
import jax.experimental.pallas.tpu as pltpu

_NT = (((1,), (1,)), ((), ()))
_NN = (((1,), (0,)), ((), ()))

_HQ, _HKV, _SK, _DH = 32, 8, 65536, 128
_REP = _HQ // _HKV
_GW = _REP * _DH
_D, _F = 512, 1792
_BK = 2048
_BPH = _SK // _BK
_T = _HKV * _BPH
_NRING = 2
_NRES = 114
_NSTR = _T - _NRES - _NRING
_RPS = -(-_NRES // _NSTR)
_NW2 = 2
_FH = _F // _NW2


def _layernorm(x):
    m = jnp.mean(x, axis=-1, keepdims=True)
    xc = x - m
    v = jnp.mean(xc * xc, axis=-1, keepdims=True)
    return xc / jnp.sqrt(v + 1e-5)


def _kernel(x_hbm, b1_hbm, k_hbm, v_hbm, wq_hbm, wo_hbm, w1_hbm, w2_hbm, o_ref,
            kpool, vpool, wq_v, wo_v, w1_v, w2_v, x_v, b1_v,
            q_s, m_s, l_s, acc_s, row_s, proj_s, cnt_s, kv_sems, w_sems):
    scale = _DH ** -0.5
    i_wq, i_wo, i_w1, i_x, i_b1, i_w2 = range(6)

    def w_copy(i):
        if i >= i_w2:
            n = i - i_w2
            src = w2_hbm.at[n * _FH:(n + 1) * _FH]
            dst = w2_v.at[n * _FH:(n + 1) * _FH]
        else:
            src, dst = ((wq_hbm, wq_v), (wo_hbm, wo_v), (w1_hbm, w1_v),
                        (x_hbm, x_v), (b1_hbm, b1_v))[i]
        return pltpu.make_async_copy(src, dst, w_sems.at[i])

    def load_desc(j):
        blk = jnp.where(j >= _T, j - _T, j)
        slot = jnp.where(
            j >= _T - _NRING, (j - (_T - _NRING)) % _NRING,
            jnp.where(j < _NSTR, j % _NRING, _NRING + (j - _NSTR)))
        return blk, slot

    def kv_copy(j, which):
        blk, slot = load_desc(j)
        src, dst = ((k_hbm, kpool), (v_hbm, vpool))[which]
        row0 = pl.multiple_of(blk * _BK, _BK)
        return pltpu.make_async_copy(
            src.at[pl.ds(row0, _BK)], dst.at[slot], kv_sems.at[which, j % _NRING])

    def start_load(j):
        kv_copy(j, 0).start()
        kv_copy(j, 1).start()

    def project(h):
        o = acc_s[h] / l_s[h]
        for r in range(_REP):
            row_s[:, r * _DH:(r + 1) * _DH] = o[r:r + 1, :]
        o = row_s[...].astype(jnp.bfloat16)
        r0 = pl.multiple_of(h * _GW, _GW)
        proj_s[...] += jnp.dot(o, wo_v[pl.ds(r0, _GW), :],
                               preferred_element_type=jnp.float32)

    def attend(blk, slot, j=None, jnext=None):
        h = blk // _BPH
        if j is not None:
            kv_copy(j, 0).wait()
        k = kpool[slot]
        q = q_s[h]
        s = jax.lax.dot_general(q, k, _NT, preferred_element_type=jnp.float32) * scale
        if jnext is not None:
            kv_copy(jnext, 0).start()
        m_old = m_s[h]
        m_new = jnp.maximum(m_old, jnp.max(s, axis=-1, keepdims=True))
        alpha = jnp.exp(m_old - m_new)
        p = jnp.exp(s - m_new)
        l_s[h] = l_s[h] * alpha + jnp.sum(p, axis=-1, keepdims=True)
        if j is not None:
            kv_copy(j, 1).wait()
        v = vpool[slot]
        acc_s[h] = acc_s[h] * alpha + jax.lax.dot_general(
            p.astype(jnp.bfloat16), v, _NN, preferred_element_type=jnp.float32)
        if jnext is not None:
            kv_copy(jnext, 1).start()
        m_s[h] = m_new
        c = cnt_s[h] + 1
        cnt_s[h] = c

        @pl.when(c == _BPH)
        def _():
            project(h)

    def reset_state():
        m_s[...] = jnp.full(m_s.shape, -jnp.inf, jnp.float32)
        l_s[...] = jnp.zeros(l_s.shape, jnp.float32)
        acc_s[...] = jnp.zeros(acc_s.shape, jnp.float32)
        proj_s[...] = jnp.zeros(proj_s.shape, jnp.float32)
        for h in range(_HKV):
            cnt_s[h] = 0

    def q_proj(xn, h0, h1):
        q = jnp.dot(xn, wq_v[:, h0 * _GW:h1 * _GW], preferred_element_type=jnp.float32)
        q = q.astype(jnp.bfloat16)
        for h in range(h0, h1):
            for r in range(_REP):
                j = (h - h0) * _REP + r
                q_s[h, r:r + 1, :] = q[:, j * _DH:(j + 1) * _DH]

    def finish_layer(x, first):
        x = x + proj_s[...]
        xn = _layernorm(x).astype(jnp.bfloat16)
        if first:
            w_copy(i_w1).wait()
        b1 = b1_v[...].astype(jnp.float32).reshape(1, _F)
        hh = jnp.dot(xn, w1_v[...], preferred_element_type=jnp.float32) + b1
        sp = jnp.log1p(jnp.exp(-jnp.abs(hh))) + jnp.maximum(hh, 0.0)
        act = (hh * jnp.tanh(sp)).astype(jnp.bfloat16)
        if not first:
            return x + jnp.dot(act, w2_v[...], preferred_element_type=jnp.float32)
        for n in range(_NW2):
            w_copy(i_w2 + n).wait()
            x = x + jnp.dot(act[:, n * _FH:(n + 1) * _FH], w2_v[n * _FH:(n + 1) * _FH, :],
                            preferred_element_type=jnp.float32)
        return x

    w_copy(i_x).start()
    w_copy(i_wq).start()
    for j in range(_NRING):
        start_load(j)
    w_copy(i_wo).start()
    w_copy(i_b1).start()

    q_s[...] = jnp.zeros(q_s.shape, q_s.dtype)
    reset_state()
    w_copy(i_x).wait()
    x0 = x_v[...].astype(jnp.float32)
    xn0 = _layernorm(x0).astype(jnp.bfloat16)
    w_copy(i_wq).wait()
    q_proj(xn0, 0, _HKV)

    def pass1(t, c):
        @pl.when(t == _BPH - 1)
        def _():
            w_copy(i_wo).wait()
            w_copy(i_b1).wait()

        blk, slot = load_desc(t)
        attend(blk, slot, t)
        jn = t + _NRING

        @pl.when(jn < _T)
        def _():
            start_load(jn)

        @pl.when(jn == _T)
        def _():
            w_copy(i_w1).start()

        @pl.when(jn == _T + 1)
        def _():
            for n in range(_NW2):
                w_copy(i_w2 + n).start()
        return c

    jax.lax.fori_loop(0, _T, pass1, 0)

    x1 = finish_layer(x0, True)
    xn1 = _layernorm(x1).astype(jnp.bfloat16)
    reset_state()

    q_proj(xn1, _HKV - 1, _HKV)
    for i in range(_NRING):
        attend(_T - _NRING + i, i, None, _T + i)
    q_proj(xn1, 0, _HKV - 1)

    def pass2(k, c):
        j = _T + k
        attend(k, k % _NRING, j)

        @pl.when(k + _NRING < _NSTR)
        def _():
            start_load(j + _NRING)

        for i in range(_RPS):
            r = k * _RPS + i

            @pl.when(r < _NRES)
            def _():
                attend(_NSTR + r, _NRING + r)
        return c

    jax.lax.fori_loop(0, _NSTR, pass2, 0)

    x2 = finish_layer(x1, False)
    o_ref[...] = x2.astype(o_ref.dtype)


@jax.jit
def pallas_interleave_layers__gqa_block_cached__dense_activation_mish__decode_kernel(
    A_x: jax.Array,
    A_k_cache: jax.Array,
    A_v_cache: jax.Array,
    A_wq: jax.Array,
    A_wo: jax.Array,
    B_x: jax.Array,
    B_w1: jax.Array,
    B_b1: jax.Array,
    B_w2: jax.Array,
):
    del B_x
    x = A_x.reshape(1, _D)
    k = A_k_cache.reshape(_HKV * _SK, _DH)
    v = A_v_cache.reshape(_HKV * _SK, _DH)
    nslot = _NRING + _NRES
    hbm = pl.BlockSpec(memory_space=pl.ANY)
    out = pl.pallas_call(
        _kernel,
        out_shape=jax.ShapeDtypeStruct((1, _D), A_x.dtype),
        in_specs=[hbm] * 8,
        out_specs=pl.BlockSpec(memory_space=pltpu.VMEM),
        scratch_shapes=[
            pltpu.VMEM((nslot, _BK, _DH), jnp.bfloat16),
            pltpu.VMEM((nslot, _BK, _DH), jnp.bfloat16),
            pltpu.VMEM((_D, _HQ * _DH), jnp.bfloat16),
            pltpu.VMEM((_HQ * _DH, _D), jnp.bfloat16),
            pltpu.VMEM((_D, _F), jnp.bfloat16),
            pltpu.VMEM((_F, _D), jnp.bfloat16),
            pltpu.VMEM((1, _D), jnp.bfloat16),
            pltpu.VMEM((_F,), jnp.bfloat16),
            pltpu.VMEM((_HKV, 8, _DH), jnp.bfloat16),
            pltpu.VMEM((_HKV, 8, 1), jnp.float32),
            pltpu.VMEM((_HKV, 8, 1), jnp.float32),
            pltpu.VMEM((_HKV, 8, _DH), jnp.float32),
            pltpu.VMEM((1, _GW), jnp.float32),
            pltpu.VMEM((1, _D), jnp.float32),
            pltpu.SMEM((_HKV,), jnp.int32),
            pltpu.SemaphoreType.DMA((2, _NRING)),
            pltpu.SemaphoreType.DMA((5 + _NW2,)),
        ],
        compiler_params=pltpu.CompilerParams(vmem_limit_bytes=128 * 1024 * 1024),
    )(x, B_b1, k, v, A_wq, A_wo, B_w1, B_w2)
    return out.reshape(A_x.shape)
```
